```python
import os as _os
_os.environ.setdefault("JAX_PLATFORMS", "cpu")
import jax
import jax.numpy as jnp

def _softmax(x, axis=-1):
    return jax.nn.softmax(x, axis=axis)
def _gelu(x):
    return jax.nn.gelu(x, approximate=True)
def _silu(x):
    return jax.nn.silu(x)
def _sigmoid(x):
    return jax.nn.sigmoid(x)
def _layernorm(x, axis=-1, eps=1e-5):
    m = jnp.mean(x, axis=axis, keepdims=True)
    v = jnp.var(x, axis=axis, keepdims=True)
    return (x - m) / jnp.sqrt(v + eps)
def _scatter_add(tgt, idx, src, axis=0):
    return tgt.at[idx].add(src)
def _segment_sum(src, seg, n):
    return jax.ops.segment_sum(src, seg, n)
class _Rng:
    def __init__(self, key):
        self._k = key
    def _next(self):
        self._k, sub = jax.random.split(self._k)
        return sub
    def normal(self, shape):
        return jax.random.normal(self._next(), shape, dtype=jnp.bfloat16)
    def randint(self, lo, hi, shape):
        return jax.random.randint(self._next(), shape, lo, hi, dtype=jnp.int32)
    def uniform(self, shape, lo=0.0, hi=1.0):
        return jax.random.uniform(self._next(), shape, jnp.bfloat16, lo, hi)
    def permutation(self, n):
        return jax.random.permutation(self._next(), n)


kernel_name = 'concat_heads__spectral_gfnet__sliding_block__prompt'

def setup_inputs():
    _rng = _Rng(jax.random.key(int.from_bytes(__import__("os").urandom(4), "little")))
    _w = (lambda a: (lambda t: t.astype(jnp.bfloat16) if jnp.issubdtype(t.dtype, jnp.floating) else t)(jnp.asarray(a)))
    def _A_setup():
        B, S, D = 1, 2048, 640
        Df = D // 2 + 1
        return {
            "x": _w((lambda *s: _rng.normal(s) * 0.05)(B, S, D)),
            "w_r": _w((lambda *s: _rng.normal(s) * 0.4)(S, Df) * 0.02),
            "w_i": _w((lambda *s: _rng.normal(s) * 0.4)(S, Df) * 0.02),
        }
    _A_in = _A_setup()

    def _B_setup():
        B, S, D = 1, 2048, 640
        return {
            "x": _w((lambda *s: _rng.normal(s) * 0.2)(B, S, D)),
            "wqkv": _w((lambda *s: _rng.normal(s) * 0.2)(D, 3 * D)),
            "wo": _w((lambda *s: _rng.normal(s) * 0.05)(D, D)),
        }
    _B_in = _B_setup()

    return {
        "A_x": _A_in["x"],
        "A_w_r": _A_in["w_r"],
        "A_w_i": _A_in["w_i"],
        "B_x": _B_in["x"],
        "B_wqkv": _B_in["wqkv"],
        "B_wo": _B_in["wo"],
    }

def reference(A_x, A_w_r, A_w_i, B_x, B_wqkv, B_wo):
    def _A_ref(x, w_r, w_i):
        B, S, D = x.shape
        X = (lambda x, axes=(-2,-1): jnp.fft.rfft2(x.astype(jnp.float32), axes=axes))(x, axes=(-2, -1))
        W = w_r + 1j * w_i
        X = X * W
        y = (lambda x, s, axes=(-2,-1): jnp.fft.irfft2(x, s=s, axes=axes).astype(jnp.bfloat16))(X, (S, D), axes=(-2, -1))
        return y

    def _B_ref(x, wqkv, wo):
        B, S, D = x.shape
        H = 32; Dh = D // H; W = 256
        qkv = (lambda x, *d: x.transpose(*d))((x @ wqkv).reshape(B, S, 3, H, Dh), 2, 0, 3, 1, 4)
        q, k, v = qkv[0], qkv[1], qkv[2]
        scores = jnp.einsum("bhqd,bhkd->bhqk", q, k) * (Dh ** -0.5)
        idx = jnp.arange(S)
        mask = (idx[:, None] - idx[None, :] >= 0) & (idx[:, None] - idx[None, :] < W)
        scores = jnp.where(mask[None, None], scores, -1e9)
        p = _softmax(scores, axis=-1)
        o = jnp.einsum("bhqk,bhkd->bhqd", p, v)
        return (lambda x, *d: x.transpose(*d))(o, 0, 2, 1, 3).reshape(B, S, D) @ wo

    a = _A_ref(A_x, A_w_r, A_w_i)
    b = _B_ref(B_x, B_wqkv, B_wo)
    return jnp.concatenate([a, b], axis=-1)
```

```python
import numpy as np
import jax
import jax.numpy as jnp
from jax.experimental import pallas as pl
from jax.experimental.pallas import tpu as pltpu

F32 = jnp.float32
BF = jnp.bfloat16
I32 = jnp.int32

S, D, DF = 2048, 640, 321
H, DH, WIN = 32, 20, 256
NEG = -1e30

C1, C2 = float(np.cos(2 * np.pi / 5)), float(np.cos(4 * np.pi / 5))
S1, S2 = float(np.sin(2 * np.pi / 5)), float(np.sin(4 * np.pi / 5))
R2 = float(np.sqrt(0.5))
QSCALE = float(DH ** -0.5 * np.log2(np.e))

_F_ALL = np.arange(DF)
_CRES = (1, 2, 0)


def _lane_maps():
    off = {(0, 0): [(0, 51)], (0, 1): [(51, 102)], (0, 2): [(102, 128)],
           (1, 0): [(51, 102)], (1, 1): [(102, 128), (0, 25)], (1, 2): [(25, 51)],
           (2, 0): [(102, 128)], (2, 1): [(25, 51)], (2, 2): [(51, 64)]}
    lanes = -np.ones((3, 128), np.int64)
    idx = np.zeros((3, 128), np.int32)
    for ci in range(3):
        c = _CRES[ci]
        fs = _F_ALL[(_F_ALL % 5 == c) | (_F_ALL % 5 == (5 - c) % 5)]
        for t in range(3):
            ft = fs[(fs >= 128 * t) & (fs < 128 * (t + 1))]
            pos = np.concatenate([np.arange(a, b) for a, b in off[(ci, t)]])
            assert len(pos) == len(ft)
            assert (lanes[ci, pos] == -1).all()
            lanes[ci, pos] = ft
            idx[t, pos] = ft - 128 * t
    return lanes, idx


_LANES, _IDX1 = _lane_maps()


def _fwd_mat(ci):
    c, f, b = _CRES[ci], _LANES[ci], np.arange(128)
    used = (f >= 0)[None, :]
    th = 2 * np.pi * np.outer(b, f) / D
    if c == 0:
        m = np.zeros((128, 256))
        m[:, :128] = np.where(used, np.cos(th), 0.0)
        m[:, 128:] = np.where(used, -np.sin(th), 0.0)
        return m
    assert used.all()
    sg = np.where(f % 5 == c, 1.0, -1.0)[None, :]
    m = np.zeros((256, 256))
    m[:128, :128] = np.cos(th)
    m[:128, 128:] = -np.sin(th)
    m[128:, :128] = sg * np.sin(th)
    m[128:, 128:] = sg * np.cos(th)
    return m


def _inv_mat(ci):
    c, f, b = _CRES[ci], _LANES[ci], np.arange(128)
    th = 2 * np.pi * np.outer(f, b) / D
    edge = (f == 0) | (f == D // 2)
    cf = np.where(f >= 0, np.where(edge, 1.0, 2.0), 0.0)[:, None] / D
    if c == 0:
        m = np.zeros((256, 128))
        m[:128] = cf * np.cos(th)
        im = -cf * np.sin(th)
        im[edge] = 0.0
        m[128:] = im
        return m
    sg = np.where(f % 5 == c, 1.0, -1.0)[:, None]
    m = np.zeros((256, 256))
    m[:128, :128] = cf * np.cos(th)
    m[128:, :128] = -cf * np.sin(th)
    m[:128, 128:] = cf * sg * np.sin(th)
    m[128:, 128:] = cf * sg * np.cos(th)
    return m


def _g_mats():
    n = np.arange(64)
    pr = 16 * (n // 8) + n % 8
    pi_ = pr + 8
    gf = np.zeros((32, 128, 128))
    gi = np.zeros((32, 128, 128))
    for k1 in range(32):
        th = 2 * np.pi * np.outer(k1 + 32 * n, n) / S
        c, s = np.cos(th), np.sin(th)
        gf[k1][np.ix_(pr, pr)] = c
        gf[k1][np.ix_(pr, pi_)] = s
        gf[k1][np.ix_(pi_, pr)] = -s
        gf[k1][np.ix_(pi_, pi_)] = c
        gi[k1][np.ix_(pr, pr)] = c.T / S
        gi[k1][np.ix_(pr, pi_)] = -s.T / S
        gi[k1][np.ix_(pi_, pr)] = s.T / S
        gi[k1][np.ix_(pi_, pi_)] = c.T / S
    order = [kp + 8 * kpp for kp in range(8) for kpp in range(4)]
    g = np.stack([np.stack([gf[order[4 * kp:4 * kp + 4]], gi[order[4 * kp:4 * kp + 4]]]) for kp in range(8)])
    return g.reshape(64 * 128, 128)


def _np_bf16(a):
    return np.asarray(a, np.float32).astype(jnp.bfloat16)


_MF = _np_bf16(np.concatenate([_fwd_mat(0), _fwd_mat(1), _fwd_mat(2)], axis=0))
_MI = _np_bf16(np.concatenate([_inv_mat(0), _inv_mat(1), _inv_mat(2)], axis=1))
_G = _np_bf16(_g_mats())
_IDX = np.repeat(_IDX1[:, None, :], 8, axis=1).reshape(24, 128).astype(np.int32)
_M32 = np.arange(32)
_TW = np.concatenate([np.cos(2 * np.pi * _M32 / 32), np.sin(2 * np.pi * _M32 / 32)]).astype(np.float32)
_ZERO = np.zeros((64,), np.int32)


def _dot(a, b):
    return jnp.dot(a, b, preferred_element_type=F32)


def _dot_nt(a, b):
    return jax.lax.dot_general(a, b, (((1,), (1,)), ((), ())), preferred_element_type=F32)


def _pack(x):
    return pltpu.bitcast(x.astype(BF), I32)


def _unpack(w):
    return pltpu.bitcast(w, BF)


def _cadd(a, b):
    return (a[0] + b[0], a[1] + b[1])


def _csub(a, b):
    return (a[0] - b[0], a[1] - b[1])


def _fft4(u, inv):
    a = _cadd(u[0], u[2])
    b = _csub(u[0], u[2])
    c = _cadd(u[1], u[3])
    d = _csub(u[1], u[3])
    o0 = _cadd(a, c)
    o2 = _csub(a, c)
    om = (b[0] + d[1], b[1] - d[0])
    op = (b[0] - d[1], b[1] + d[0])
    return [o0, op, o2, om] if inv else [o0, om, o2, op]


def _fft8(u, inv):
    e = _fft4([u[0], u[2], u[4], u[6]], inv)
    o = _fft4([u[1], u[3], u[5], u[7]], inv)
    out = [None] * 8
    out[0] = _cadd(e[0], o[0])
    out[4] = _csub(e[0], o[0])
    p = (o[1][0] + o[1][1]) * R2
    m = (o[1][1] - o[1][0]) * R2
    if not inv:
        out[1] = (e[1][0] + p, e[1][1] + m)
        out[5] = (e[1][0] - p, e[1][1] - m)
        out[2] = (e[2][0] + o[2][1], e[2][1] - o[2][0])
        out[6] = (e[2][0] - o[2][1], e[2][1] + o[2][0])
    else:
        out[1] = (e[1][0] - m, e[1][1] + p)
        out[5] = (e[1][0] + m, e[1][1] - p)
        out[2] = (e[2][0] - o[2][1], e[2][1] + o[2][0])
        out[6] = (e[2][0] + o[2][1], e[2][1] - o[2][0])
    p = (o[3][0] + o[3][1]) * R2
    m = (o[3][1] - o[3][0]) * R2
    if not inv:
        out[3] = (e[3][0] + m, e[3][1] - p)
        out[7] = (e[3][0] - m, e[3][1] + p)
    else:
        out[3] = (e[3][0] - p, e[3][1] - m)
        out[7] = (e[3][0] + p, e[3][1] + m)
    return out


def _l1_iter(i, x_ref, mf_ref, tw_ref, yp_ref):
    al = i // 4
    bc = i % 4
    xs = [x_ref[j, i] for j in range(8)]
    x = jnp.concatenate(xs, axis=0).astype(F32)
    x0, x1, x2, x3, x4 = [x[:, 128 * a:128 * a + 128] for a in range(5)]
    t1 = x1 + x4
    t2 = x2 + x3
    t3 = x1 - x4
    t4 = x2 - x3
    y0 = x0 + t1 + t2
    y1r = x0 + C1 * t1 + C2 * t2
    y2r = x0 + C2 * t1 + C1 * t2
    y1i = -(S1 * t3 + S2 * t4)
    y2i = S1 * t4 - S2 * t3
    lhs = [jnp.concatenate([y1r, y1i], axis=1).astype(BF),
           jnp.concatenate([y2r, y2i], axis=1).astype(BF),
           y0.astype(BF)]
    ws = [mf_ref[0:256, :], mf_ref[256:512, :], mf_ref[512:640, :]]
    for c in range(3):
        z = _dot(lhs[c], ws[c])
        u = [(z[16 * j:16 * j + 16, 0:128], z[16 * j:16 * j + 16, 128:256]) for j in range(8)]
        o = _fft8(u, False)
        for kp in range(8):
            re, im = o[kp]
            if kp > 0:
                m = (al * kp) % 32
                cs = tw_ref[m]
                sn = tw_ref[32 + m]
                re, im = re * cs + im * sn, im * cs - re * sn
            blk = jnp.concatenate([re[0:8], im[0:8], re[8:16], im[8:16]], axis=0)
            r0 = pl.multiple_of(((c * 8 + kp) * 4 + al) * 128 + 32 * bc, 32)
            yp_ref[pl.ds(r0, 32), :] = blk


def _l2_fwd(u, yp_ref, g_ref, wp_ref):
    c = u // 8
    kp = u % 8
    base = pl.multiple_of(u * 512, 512)
    ys = [yp_ref[pl.ds(base + al * 128, 128), :] for al in range(4)]
    outs = [[None] * 8 for _ in range(4)]
    for g in range(8):
        o = _fft4([(ys[al][16 * g:16 * g + 8], ys[al][16 * g + 8:16 * g + 16]) for al in range(4)], False)
        for kpp in range(4):
            outs[kpp][g] = jnp.concatenate([o[kpp][0], o[kpp][1]], axis=0)
    vsl = []
    for kpp in range(4):
        k1 = kp + 8 * kpp
        yw = jnp.concatenate(outs[kpp], axis=0).astype(BF)
        gf = g_ref[pl.ds(pl.multiple_of((kp * 8 + kpp) * 128, 128), 128), :]
        xx = _dot(gf, yw)
        w = wp_ref[pl.ds(pl.multiple_of((c * 32 + k1) * 128, 128), 128), :]
        vs = []
        for g in range(8):
            xr, xi = xx[16 * g:16 * g + 8], xx[16 * g + 8:16 * g + 16]
            wr, wi = w[16 * g:16 * g + 8], w[16 * g + 8:16 * g + 16]
            vs += [xr * wr - xi * wi, xr * wi + xi * wr]
        vsl.append(jnp.concatenate(vs, axis=0).astype(BF))
    return vsl


def _l2_inv(u, vsl, g_ref):
    kp = u % 8
    us = []
    for kpp in range(4):
        gi = g_ref[pl.ds(pl.multiple_of((kp * 8 + 4 + kpp) * 128, 128), 128), :]
        us.append(_dot(gi, vsl[kpp]))
    return us


def _l2_fin(u, us, up_ref):
    base = pl.multiple_of(u * 512, 512)
    res = [[None] * 8 for _ in range(4)]
    for g in range(8):
        o = _fft4([(us[kpp][16 * g:16 * g + 8], us[kpp][16 * g + 8:16 * g + 16]) for kpp in range(4)], True)
        for al in range(4):
            res[al][g] = jnp.concatenate([o[al][0], o[al][1]], axis=0)
    for al in range(4):
        up_ref[pl.ds(base + al * 128, 128), :] = jnp.concatenate(res[al], axis=0)


def _l3_a(i, up_ref, mi_ref, tw_ref):
    al = i // 4
    bc = i % 4
    vs = []
    for c in range(3):
        u = []
        for kp in range(8):
            r0 = pl.multiple_of(((c * 8 + kp) * 4 + al) * 128 + 32 * bc, 32)
            blk = up_ref[pl.ds(r0, 32), :]
            re = jnp.concatenate([blk[0:8], blk[16:24]], axis=0)
            im = jnp.concatenate([blk[8:16], blk[24:32]], axis=0)
            if kp > 0:
                m = (al * kp) % 32
                cs = tw_ref[m]
                sn = tw_ref[32 + m]
                re, im = re * cs - im * sn, im * cs + re * sn
            u.append((re, im))
        o = _fft8(u, True)
        zr = jnp.concatenate([o[j][0] for j in range(8)], axis=0)
        zi = jnp.concatenate([o[j][1] for j in range(8)], axis=0)
        lhs = jnp.concatenate([zr, zi], axis=1).astype(BF)
        w = mi_ref[:, 256 * c:256 * c + 256] if c < 2 else mi_ref[:, 512:640]
        vs.append(_dot(lhs, w))
    return vs


def _l3_b(i, vs, out_ref):
    v1r, v1i = vs[0][:, :128], vs[0][:, 128:]
    v2r, v2i = vs[1][:, :128], vs[1][:, 128:]
    v0 = vs[2]
    pa = C1 * v1r + C2 * v2r
    pb = C2 * v1r + C1 * v2r
    qa = S1 * v1i + S2 * v2i
    qb = S2 * v1i - S1 * v2i
    ea = v0 + pa
    eb = v0 + pb
    ys = [v0 + v1r + v2r, ea - qa, eb - qb, eb + qb, ea + qa]
    y = jnp.concatenate(ys, axis=1).astype(BF)
    for j in range(8):
        r0 = pl.multiple_of(256 * j + 16 * i, 16)
        out_ref[pl.ds(r0, 16), 0:D] = y[16 * j:16 * j + 16]


def _wprep_iter(hi3, w_ref, idx_ref, wp_ref, part):
    lane = jax.lax.broadcasted_iota(I32, (128, 128), 1)
    sub = jax.lax.broadcasted_iota(I32, (8, 128), 0)
    srt = []
    for t in range(3):
        halves = []
        for kt in range(2):
            k0 = pl.multiple_of(hi3 * 256 + kt * 128, 128)
            if t < 2:
                blk = w_ref[128 * t:128 * t + 128, pl.ds(k0, 128)]
            else:
                blk = jnp.concatenate([w_ref[256:DF, pl.ds(k0, 128)], jnp.zeros((384 - DF, 128), BF)], axis=0)
            halves.append(pltpu.bitcast(blk.T, I32))
        words = jnp.concatenate(halves, axis=0)
        idx = jnp.broadcast_to(idx_ref[8 * t:8 * t + 1, :], (128, 128))
        srt.append(jnp.take_along_axis(words, idx, axis=1))
    for c in range(3):
        if c == 0:
            t = jnp.where(lane < 51, srt[0], jnp.where(lane < 102, srt[1], srt[2]))
        elif c == 1:
            t = jnp.where((lane >= 51) & (lane < 102), srt[0], jnp.where((lane >= 25) & (lane < 51), srt[2], srt[1]))
        else:
            t = jnp.where(lane >= 102, srt[0], jnp.where(lane < 51, srt[1], srt[2]))
        for bit4 in range(2):
            v = [t[8 * (bit4 + 2 * m):8 * (bit4 + 2 * m) + 8] for m in range(8)]
            for s_ in range(3):
                sh = 1 << s_
                nv = [None] * 8
                lo_mask = (sub & sh) == 0
                for m in range(8):
                    if m & sh:
                        continue
                    a_, b_ = v[m], v[m + sh]
                    ra = pltpu.roll(a_, 8 - sh, axis=0)
                    rb = pltpu.roll(b_, sh, axis=0)
                    nv[m] = jnp.where(lo_mask, a_, rb)
                    nv[m + sh] = jnp.where(lo_mask, ra, b_)
                v = nv
            for mp in range(8):
                lo = pltpu.bitcast(v[mp] << 16, F32)
                hi = pltpu.bitcast(v[mp] & jnp.int32(-65536), F32)
                for half, val in ((0, lo), (1, hi)):
                    k1 = half + 2 * mp + 16 * bit4
                    rr = pl.multiple_of((c * 32 + k1) * 128 + 16 * hi3 + 8 * part, 8)
                    wp_ref[pl.ds(rr, 8), :] = val


def _kproj(i, xb_ref, wk_ref, k32_ref):
    r0 = pl.multiple_of(i * 128, 128)
    z = _dot(xb_ref[pl.ds(r0, 128), :], wk_ref[...])
    w = _pack(z)
    lane = jax.lax.broadcasted_iota(I32, (64, 128), 1)
    t = [w[:, 128 * a:128 * a + 128] for a in range(5)]
    mix = [jnp.where(lane >= 64, t[a], t[a + 1]) for a in range(4)]
    k32_ref[pl.ds(pl.multiple_of(i * 64, 64), 64), :] = jnp.concatenate(t + mix, axis=1)


def _qproj(i, xb_ref, wqt_ref, qt32_ref):
    r0 = pl.multiple_of(i * 128, 128)
    z = _dot_nt(_unpack(wqt_ref[...]), xb_ref[pl.ds(r0, 128), :])
    qt32_ref[:, pl.ds(r0, 128)] = _pack(z * QSCALE)


def _vproj(i, xb_ref, wvt_ref, vt32_ref):
    r0 = pl.multiple_of(i * 128, 128)
    z = _dot_nt(_unpack(wvt_ref[...]), xb_ref[pl.ds(r0, 128), :])
    ones8 = jnp.where(jax.lax.broadcasted_iota(I32, (8, 128), 0) == 0, 1.0, 0.0).astype(F32)
    pieces = []
    for m in range(H // 2):
        pieces += [z[40 * m:40 * m + 24], ones8, z[40 * m + 16:40 * m + 40], ones8]
    vt32_ref[:, pl.ds(r0, 128)] = _pack(jnp.concatenate(pieces, axis=0))


def _head_tile(h):
    lo = DH * h
    t = lo // 128
    if lo % 128 + DH <= 128:
        return False, t
    return True, t


def _get_wq(qt32_ref, h, q0):
    mix, t = _head_tile(h)
    rowi = jax.lax.broadcasted_iota(I32, (64, 128), 0)
    rlo = (DH * h - 128 * t) // 2
    if not mix:
        w = qt32_ref[64 * t:64 * t + 64, pl.ds(q0, 128)]
        msk = (rowi >= rlo) & (rowi < rlo + DH // 2)
        kt = t
    else:
        w = jnp.concatenate([qt32_ref[64 * t + 64:64 * t + 96, pl.ds(q0, 128)],
                             qt32_ref[64 * t + 32:64 * t + 64, pl.ds(q0, 128)]], axis=0)
        msk = (rowi >= rlo) | (rowi < rlo + DH // 2 - 64)
        kt = 5 + t
    return kt, _unpack(jnp.where(msk, w, 0))


def _s1(j, g, nb, buf, z, k32_ref, qt32_ref):
    q0 = pl.multiple_of(j * 128, 128)
    r = jax.lax.broadcasted_iota(I32, (128, 128), 0)
    c = jax.lax.broadcasted_iota(I32, (128, 128), 1)
    upper = r > c
    ms = [None] * 4
    zz = pl.multiple_of(z * 8, 8)
    for b in range(3 - nb, 3):
        for a in range(4):
            h = 4 * g + a
            kt, wq = _get_wq(qt32_ref, h, q0)
            k0 = pl.multiple_of((j - 2 + b) * 64, 64)
            kb = _unpack(k32_ref[pl.ds(k0, 64), 128 * kt:128 * kt + 128])
            s = _dot(kb, wq)
            if b == 0:
                s = jnp.where(upper, s, NEG)
            if b == 2:
                s = jnp.where(upper, NEG, s)
            buf[pl.ds(zz + (a * 3 + b) * 128, 128), :] = s
            mb = jnp.max(s.reshape(16, 8, 128), axis=0)
            ms[a] = mb if ms[a] is None else jnp.maximum(ms[a], mb)
    return [jnp.max(m, axis=0, keepdims=True) for m in ms]


def _s2(j, g, nb, buf, z, ms, vt32_ref, aot_ref):
    sub = jax.lax.broadcasted_iota(I32, (8, 128), 0)
    acc = [None] * 4
    zz = pl.multiple_of(z * 8, 8)
    for b in range(3 - nb, 3):
        k0 = pl.multiple_of((j - 2 + b) * 128, 128)
        for a in range(4):
            h = 4 * g + a
            p = jnp.exp2(buf[pl.ds(zz + (a * 3 + b) * 128, 128), :] - ms[a]).astype(BF)
            vt = _unpack(vt32_ref[16 * h:16 * h + 16, pl.ds(k0, 128)])
            d = _dot(vt, p)
            acc[a] = d if acc[a] is None else acc[a] + d
    os_ = [o[0:24, :] * (1.0 / o[24:25, :]) for o in acc]
    blks = []
    for a in (0, 2):
        e, od = os_[a], os_[a + 1]
        blks += [e[0:16], jnp.where(sub < 4, e[16:24], od[0:8]), od[8:24]]
    aot_ref[80 * g:80 * g + 80, :] = jnp.concatenate(blks, axis=0)


def _outproj(j, aot_ref, wo_ref, out_ref):
    ao = jnp.concatenate([aot_ref[128 * t:128 * t + 128, :].T for t in range(5)], axis=1).astype(BF)
    z = _dot(ao, wo_ref[...])
    out_ref[pl.ds(pl.multiple_of(j * 128, 128), 128), D:2 * D] = z.astype(BF)


def _kernel(tw_ref, z_ref, idx_ref,
            xa_hbm, wr_hbm, wi_hbm, xb_hbm, wqkv_hbm, wo_hbm, g_hbm, mf_hbm, mi_hbm, out_hbm,
            xa_v, wr_v, wi_v, xb_v, wq_v, wk_v, wv_v, wo_v, g_v, mf_ref, mi_ref,
            wqt_v, wvt_v, k32, qt32, vt32, aot, sbuf0, sbuf1,
            yp, up, wp, ostage, sems, csem, gsem, osem):
    def cp(src, dst, k):
        return pltpu.make_async_copy(src, dst, sems.at[k])

    c_wk = cp(wqkv_hbm.at[:, D:2 * D], wk_v, 0)
    c_wq = cp(wqkv_hbm.at[:, 0:D], wq_v, 1)
    c_wv = cp(wqkv_hbm.at[:, 2 * D:3 * D], wv_v, 2)
    c_wo = cp(wo_hbm, wo_v, 3)
    c_mf = cp(mf_hbm, mf_ref, 4)
    c_mi = cp(mi_hbm, mi_ref, 5)

    def chunk(i):
        r = pl.ds(pl.multiple_of(i * 256, 256), 256)
        m = pl.ds(pl.multiple_of(i * 2, 2), 2)
        return (pltpu.make_async_copy(xb_hbm.at[r], xb_v.at[r], csem.at[4 * i]),
                pltpu.make_async_copy(xa_hbm.at[:, m], xa_v.at[:, m], csem.at[4 * i + 1]),
                pltpu.make_async_copy(wr_hbm.at[:, r], wr_v.at[:, r], csem.at[4 * i + 2]),
                pltpu.make_async_copy(wi_hbm.at[:, r], wi_v.at[:, r], csem.at[4 * i + 3]))

    def gchunk(kp):
        r = pl.ds(pl.multiple_of(kp * 1024, 1024), 1024)
        return pltpu.make_async_copy(g_hbm.at[r], g_v.at[r], gsem.at[kp])

    def loop(n, f):
        jax.lax.fori_loop(0, n, lambda i, c_: (f(i), c_)[1], 0)

    c_wk.start()
    ch0 = chunk(0)
    ch0[0].start()
    c_mf.start()
    for c_ in ch0[1:]:
        c_.start()

    c_wk.wait()
    for c_ in chunk(1):
        c_.start()
    c_mf.wait()

    def ph1(i):
        @pl.when(i < 6)
        def _():
            for c_ in chunk(i + 2):
                c_.start()

        pl.when(i == 4)(c_wq.start)
        pl.when(i == 6)(gchunk(0).start)
        pl.when(i == 7)(gchunk(1).start)
        for c_ in chunk(i):
            c_.wait()
        for t in range(2):
            _kproj(2 * i + t, xb_v, wk_v, k32)
            _l1_iter(2 * i + t, xa_v, mf_ref, tw_ref, yp)
        _wprep_iter(i, wr_v, idx_ref, wp, 0)
        _wprep_iter(i, wi_v, idx_ref, wp, 1)
    loop(8, ph1)

    c_wq.wait()
    wqt_v[...] = pltpu.bitcast(wq_v[...].T, I32)

    def ph2(kp):
        @pl.when(kp < 6)
        def _():
            gchunk(kp + 2).start()

        pl.when(kp == 2)(c_wv.start)
        pl.when(kp == 4)(c_mi.start)
        pl.when(kp == 5)(c_wo.start)
        gchunk(kp).wait()
        st = [_l2_fwd(c * 8 + kp, yp, g_v, wp) for c in range(3)]
        _qproj(2 * kp, xb_v, wqt_v, qt32)
        us = [_l2_inv(c * 8 + kp, st[c], g_v) for c in range(3)]
        _qproj(2 * kp + 1, xb_v, wqt_v, qt32)
        for c in range(3):
            _l2_fin(c * 8 + kp, us[c], up)
    loop(8, ph2)

    c_wv.wait()
    wvt_v[...] = pltpu.bitcast(wv_v[...].T, I32)
    c_mi.wait()
    ost4 = ostage.reshape(8, 16, 16, 2 * D)
    out4 = out_hbm.reshape(8, 16, 16, 2 * D)

    def out_a(i):
        m = pl.ds(pl.multiple_of(i * 2, 2), 2)
        return pltpu.make_async_copy(ost4.at[:, m, :, 0:D], out4.at[:, m, :, 0:D], osem.at[0])

    def ph3(i):
        _vproj(2 * i, xb_v, wvt_v, vt32)
        va = _l3_a(2 * i, up, mi_ref, tw_ref)
        _vproj(2 * i + 1, xb_v, wvt_v, vt32)
        vb = _l3_a(2 * i + 1, up, mi_ref, tw_ref)
        _l3_b(2 * i, va, ostage)
        _l3_b(2 * i + 1, vb, ostage)
        out_a(i).start()
    loop(8, ph3)

    c_wo.wait()
    bufs = (sbuf0, sbuf1)
    zc = [0]

    def oz():
        zc[0] += 1
        return z_ref[zc[0] % 64]

    def out_copy(j):
        rows = pl.ds(pl.multiple_of(j * 128, 128), 128)
        return pltpu.make_async_copy(ostage.at[rows, D:2 * D], out_hbm.at[rows, D:2 * D], osem.at[1])

    def body(j, nb, nb_next, ms, first, last):
        for g in range(8):
            if g < 7:
                ms_n = _s1(j, g + 1, nb, bufs[(g + 1) % 2], oz(), k32, qt32)
            elif not last:
                ms_n = _s1(j + 1, 0, nb_next, bufs[0], oz(), k32, qt32)
            else:
                ms_n = None
            if g == 0 and not first:
                _outproj(j - 1, aot, wo_v, ostage)
                out_copy(j - 1).start()
            _s2(j, g, nb, bufs[g % 2], oz(), ms, vt32, aot)
            ms = ms_n
        return ms

    ms = _s1(0, 0, 1, bufs[0], oz(), k32, qt32)
    ms = body(0, 1, 2, ms, True, False)
    ms = body(1, 2, 3, ms, False, False)
    ms = jax.lax.fori_loop(2, 15, lambda j, m: tuple(body(j, 3, 3, list(m), False, False)), tuple(ms))
    body(15, 3, 3, list(ms), False, True)
    _outproj(15, aot, wo_v, ostage)
    out_copy(15).start()
    for j in range(8):
        out_a(j).wait()
    for j in range(16):
        out_copy(j).wait()


@jax.jit
def pallas_concat_heads__spectral_gfnet__sliding_block__prompt_kernel(
    A_x: jax.Array,
    A_w_r: jax.Array,
    A_w_i: jax.Array,
    B_x: jax.Array,
    B_wqkv: jax.Array,
    B_wo: jax.Array,
):
    smem = pl.BlockSpec(memory_space=pltpu.SMEM)
    vmem = pl.BlockSpec(memory_space=pltpu.VMEM)
    hbm = pl.BlockSpec(memory_space=pltpu.HBM)
    out = pl.pallas_call(
        _kernel,
        out_shape=jax.ShapeDtypeStruct((S, 2 * D), BF),
        in_specs=[smem, smem, vmem] + [hbm] * 9,
        out_specs=hbm,
        scratch_shapes=[
            pltpu.VMEM((8, 16, 16, D), BF), pltpu.VMEM((DF, S), BF), pltpu.VMEM((DF, S), BF), pltpu.VMEM((S, D), BF),
            pltpu.VMEM((D, D), BF), pltpu.VMEM((D, D), BF), pltpu.VMEM((D, D), BF), pltpu.VMEM((D, D), BF),
            pltpu.VMEM((64 * 128, 128), BF), pltpu.VMEM((D, 256), BF), pltpu.VMEM((256, D), BF),
            pltpu.VMEM((D // 2, D), I32), pltpu.VMEM((D // 2, D), I32),
            pltpu.VMEM((S // 2, 9 * 128), I32), pltpu.VMEM((D // 2, S), I32), pltpu.VMEM((512, S), I32),
            pltpu.VMEM((D, 128), F32),
            pltpu.VMEM((12 * 128, 128), F32), pltpu.VMEM((12 * 128, 128), F32),
            pltpu.VMEM((96 * 128, 128), F32), pltpu.VMEM((96 * 128, 128), F32), pltpu.VMEM((96 * 128, 128), F32),
            pltpu.VMEM((S, 2 * D), BF),
            pltpu.SemaphoreType.DMA((6,)), pltpu.SemaphoreType.DMA((32,)), pltpu.SemaphoreType.DMA((8,)),
            pltpu.SemaphoreType.DMA((2,)),
        ],
        compiler_params=pltpu.CompilerParams(vmem_limit_bytes=110 * 1024 * 1024),
    )(_TW, _ZERO, _IDX,
      A_x.reshape(8, 16, 16, D), A_w_r.T, A_w_i.T, B_x.reshape(S, D), B_wqkv, B_wo, _G, _MF, _MI)
    return out.reshape(1, S, 2 * D)
```

```python
import functools
import numpy as np
import jax
import jax.numpy as jnp
from jax.experimental import pallas as pl
from jax.experimental.pallas import tpu as pltpu

F32 = jnp.float32
BF = jnp.bfloat16
I32 = jnp.int32

S, D, DF = 2048, 640, 321
H, DH, WIN = 32, 20, 256
NEG = -1e30

C1, C2 = float(np.cos(2 * np.pi / 5)), float(np.cos(4 * np.pi / 5))
S1, S2 = float(np.sin(2 * np.pi / 5)), float(np.sin(4 * np.pi / 5))
R2 = float(np.sqrt(0.5))
QSCALE = float(DH ** -0.5 * np.log2(np.e))

_F_ALL = np.arange(DF)
_CRES = (1, 2, 0)


def _lane_maps():
    off = {(0, 0): [(0, 51)], (0, 1): [(51, 102)], (0, 2): [(102, 128)],
           (1, 0): [(51, 102)], (1, 1): [(102, 128), (0, 25)], (1, 2): [(25, 51)],
           (2, 0): [(102, 128)], (2, 1): [(25, 51)], (2, 2): [(51, 64)]}
    lanes = -np.ones((3, 128), np.int64)
    idx = np.zeros((3, 128), np.int32)
    for ci in range(3):
        c = _CRES[ci]
        fs = _F_ALL[(_F_ALL % 5 == c) | (_F_ALL % 5 == (5 - c) % 5)]
        for t in range(3):
            ft = fs[(fs >= 128 * t) & (fs < 128 * (t + 1))]
            pos = np.concatenate([np.arange(a, b) for a, b in off[(ci, t)]])
            assert len(pos) == len(ft)
            assert (lanes[ci, pos] == -1).all()
            lanes[ci, pos] = ft
            idx[t, pos] = ft - 128 * t
    return lanes, idx


_LANES, _IDX1 = _lane_maps()


def _fwd_mat(ci):
    c, f, b = _CRES[ci], _LANES[ci], np.arange(128)
    used = (f >= 0)[None, :]
    th = 2 * np.pi * np.outer(b, f) / D
    if c == 0:
        m = np.zeros((128, 256))
        m[:, :128] = np.where(used, np.cos(th), 0.0)
        m[:, 128:] = np.where(used, -np.sin(th), 0.0)
        return m
    assert used.all()
    sg = np.where(f % 5 == c, 1.0, -1.0)[None, :]
    m = np.zeros((256, 256))
    m[:128, :128] = np.cos(th)
    m[:128, 128:] = -np.sin(th)
    m[128:, :128] = sg * np.sin(th)
    m[128:, 128:] = sg * np.cos(th)
    return m


def _inv_mat(ci):
    c, f, b = _CRES[ci], _LANES[ci], np.arange(128)
    th = 2 * np.pi * np.outer(f, b) / D
    edge = (f == 0) | (f == D // 2)
    cf = np.where(f >= 0, np.where(edge, 1.0, 2.0), 0.0)[:, None] / D
    if c == 0:
        m = np.zeros((256, 128))
        m[:128] = cf * np.cos(th)
        im = -cf * np.sin(th)
        im[edge] = 0.0
        m[128:] = im
        return m
    sg = np.where(f % 5 == c, 1.0, -1.0)[:, None]
    m = np.zeros((256, 256))
    m[:128, :128] = cf * np.cos(th)
    m[128:, :128] = -cf * np.sin(th)
    m[:128, 128:] = cf * sg * np.sin(th)
    m[128:, 128:] = cf * sg * np.cos(th)
    return m


def _g_mats():
    n = np.arange(64)
    pr = 16 * (n // 8) + n % 8
    pi_ = pr + 8
    gf = np.zeros((32, 128, 128))
    gi = np.zeros((32, 128, 128))
    for k1 in range(32):
        th = 2 * np.pi * np.outer(k1 + 32 * n, n) / S
        c, s = np.cos(th), np.sin(th)
        gf[k1][np.ix_(pr, pr)] = c
        gf[k1][np.ix_(pr, pi_)] = s
        gf[k1][np.ix_(pi_, pr)] = -s
        gf[k1][np.ix_(pi_, pi_)] = c
        gi[k1][np.ix_(pr, pr)] = c.T / S
        gi[k1][np.ix_(pr, pi_)] = -s.T / S
        gi[k1][np.ix_(pi_, pr)] = s.T / S
        gi[k1][np.ix_(pi_, pi_)] = c.T / S
    order = [kp + 8 * kpp for kp in range(8) for kpp in range(4)]
    g = np.stack([np.stack([gf[order[4 * kp:4 * kp + 4]], gi[order[4 * kp:4 * kp + 4]]]) for kp in range(8)])
    return g.reshape(64 * 128, 128)


def _np_bf16(a):
    b = np.asarray(a, np.float32).astype(jnp.bfloat16).view(np.uint16).astype(np.uint32)
    return (b[0::2] | (b[1::2] << 16)).view(np.int32)


_C0L = np.where(_LANES[2] >= 0)[0]
_C0F = _LANES[2][_C0L]
_C0IM = [(l, f) for l, f in zip(_C0L, _C0F) if f not in (0, D // 2)]
_C0REST = np.where(_LANES[2] < 0)[0]
assert len(_C0IM) == len(_C0REST) == 63
_IDXF = np.zeros(128, np.int32)
_IDXI = np.zeros(128, np.int32)
for (_l, _f), _pk in zip(_C0IM, _C0REST):
    _IDXF[_l] = _pk
    _IDXI[_pk] = _l
_EDGE = [int(_l) for _l, _f in zip(_C0L, _C0F) if _f in (0, D // 2)]


def _fwd_mat0():
    b = np.arange(128)[:, None]
    m = np.zeros((128, 128))
    m[:, _C0L] = np.cos(2 * np.pi * b * _C0F[None, :] / D)
    for (_l, _f), _pk in zip(_C0IM, _C0REST):
        m[:, _pk] = -np.sin(2 * np.pi * b[:, 0] * _f / D)
    return m


def _inv_mat0():
    b = np.arange(128)
    m = np.zeros((128, 128))
    for _l, _f in zip(_C0L, _C0F):
        m[_l] = (1.0 if _f in (0, D // 2) else 2.0) / D * np.cos(2 * np.pi * _f * b / D)
    for (_l, _f), _pk in zip(_C0IM, _C0REST):
        m[_pk] = -2.0 / D * np.sin(2 * np.pi * _f * b / D)
    return m


_C0RANGES = []
for _l in _C0L:
    if _C0RANGES and _C0RANGES[-1][1] == _l:
        _C0RANGES[-1][1] = int(_l) + 1
    else:
        _C0RANGES.append([int(_l), int(_l) + 1])
_MF0 = np.concatenate([_fwd_mat0(), np.zeros((128, 128))], axis=1)
_MI0 = _inv_mat0()
def _gauss(ci):
    m = _fwd_mat(ci)
    c_, s2_ = m[:128, :128], m[128:, :128]
    t_ = m[:128, 128:] + m[128:, 128:]
    sg = np.where(_LANES[ci] % 5 == _CRES[ci], 1.0, -1.0)
    return np.concatenate([c_, s2_, t_], axis=1), sg


_GA, _SGA = _gauss(0)
_GB, _SGB = _gauss(1)
_MF = _np_bf16(np.concatenate([_GA, _GB, np.concatenate([_fwd_mat0(), np.zeros((128, 256))], axis=1)], axis=0))
def _gauss_inv(ci):
    m = _inv_mat(ci)
    c_, ss_ = m[:128, :128], m[:128, 128:]
    return np.concatenate([c_, ss_, c_ + ss_], axis=1)


_MI = _np_bf16(np.concatenate([_gauss_inv(0), _gauss_inv(1), _MI0], axis=1))
_G = _np_bf16(_g_mats())
_IDX = np.repeat(np.concatenate([_IDX1, _IDXF[None], _IDXI[None], _SGA.astype(np.float32).view(np.int32)[None], _SGB.astype(np.float32).view(np.int32)[None]])[:, None, :], 8, axis=1).reshape(56, 128).astype(np.int32)
_M32 = np.arange(32)
_TW = np.concatenate([np.cos(2 * np.pi * _M32 / 32), np.sin(2 * np.pi * _M32 / 32)]).astype(np.float32)
NZ = 16


def _dot(a, b):
    return jnp.dot(a, b, preferred_element_type=F32)


def _dot_nt(a, b):
    return jax.lax.dot_general(a, b, (((1,), (1,)), ((), ())), preferred_element_type=F32)


def _pack(x):
    return pltpu.bitcast(x.astype(BF), I32)


def _unpack(w):
    return pltpu.bitcast(w, BF)


def _cadd(a, b):
    return (a[0] + b[0], a[1] + b[1])


def _csub(a, b):
    return (a[0] - b[0], a[1] - b[1])


def _fft4(u, inv):
    a = _cadd(u[0], u[2])
    b = _csub(u[0], u[2])
    c = _cadd(u[1], u[3])
    d = _csub(u[1], u[3])
    o0 = _cadd(a, c)
    o2 = _csub(a, c)
    om = (b[0] + d[1], b[1] - d[0])
    op = (b[0] - d[1], b[1] + d[0])
    return [o0, op, o2, om] if inv else [o0, om, o2, op]


def _fft8(u, inv):
    e = _fft4([u[0], u[2], u[4], u[6]], inv)
    o = _fft4([u[1], u[3], u[5], u[7]], inv)
    out = [None] * 8
    out[0] = _cadd(e[0], o[0])
    out[4] = _csub(e[0], o[0])
    p = (o[1][0] + o[1][1]) * R2
    m = (o[1][1] - o[1][0]) * R2
    if not inv:
        out[1] = (e[1][0] + p, e[1][1] + m)
        out[5] = (e[1][0] - p, e[1][1] - m)
        out[2] = (e[2][0] + o[2][1], e[2][1] - o[2][0])
        out[6] = (e[2][0] - o[2][1], e[2][1] + o[2][0])
    else:
        out[1] = (e[1][0] - m, e[1][1] + p)
        out[5] = (e[1][0] + m, e[1][1] - p)
        out[2] = (e[2][0] - o[2][1], e[2][1] + o[2][0])
        out[6] = (e[2][0] + o[2][1], e[2][1] - o[2][0])
    p = (o[3][0] + o[3][1]) * R2
    m = (o[3][1] - o[3][0]) * R2
    if not inv:
        out[3] = (e[3][0] + m, e[3][1] - p)
        out[7] = (e[3][0] - m, e[3][1] + p)
    else:
        out[3] = (e[3][0] - p, e[3][1] - m)
        out[7] = (e[3][0] + p, e[3][1] + m)
    return out


def _l1_a(i, x_ref, mf_ref, idx_ref):
    xs = [x_ref[j, i] for j in range(8)]
    x = jnp.concatenate(xs, axis=0).astype(F32)
    x0, x1, x2, x3, x4 = [x[:, 128 * a:128 * a + 128] for a in range(5)]
    t1 = x1 + x4
    t2 = x2 + x3
    t3 = x1 - x4
    t4 = x2 - x3
    y0 = x0 + t1 + t2
    y1r = x0 + C1 * t1 + C2 * t2
    y2r = x0 + C2 * t1 + C1 * t2
    y1i = -(S1 * t3 + S2 * t4)
    y2i = S1 * t4 - S2 * t3
    z0 = _dot(y0.astype(BF), _unpack(mf_ref[128:192, 0:128]))
    zs = []
    for c, (yr, yi) in enumerate(((y1r, y1i), (y2r, y2i))):
        p1 = _dot(yr.astype(BF), _unpack(mf_ref[64 * c:64 * c + 64, 0:128]))
        p2 = _dot(yi.astype(BF), _unpack(mf_ref[64 * c:64 * c + 64, 128:256]))
        p3 = _dot((yr + yi).astype(BF), _unpack(mf_ref[64 * c:64 * c + 64, 256:384]))
        sg = pltpu.bitcast(idx_ref[40 + 8 * c:48 + 8 * c, :], F32)
        sg = jnp.concatenate([sg] * 16, axis=0)
        zs.append(jnp.concatenate([p1 + p2, p3 + sg * (p2 - p1)], axis=1))
    lane = jax.lax.broadcasted_iota(I32, (128, 128), 1)
    im = jnp.take_along_axis(z0, jnp.broadcast_to(idx_ref[24:25, :], (128, 128)), axis=1)
    im = jnp.where((lane == _EDGE[0]) | (lane == _EDGE[1]), 0.0, im)
    return zs + [jnp.concatenate([z0, im], axis=1)]


def _l1_b(i, zs, tw_ref, yp_ref):
    al = i // 4
    bc = i % 4
    for c in range(3):
        z = zs[c]
        u = [(z[16 * j:16 * j + 16, 0:128], z[16 * j:16 * j + 16, 128:256]) for j in range(8)]
        o = _fft8(u, False)
        for kp in range(8):
            re, im = o[kp]
            blk = jnp.concatenate([re[0:8], im[0:8], re[8:16], im[8:16]], axis=0)
            r0 = pl.multiple_of(((c * 8 + kp) * 4 + al) * 128 + 32 * bc, 32)
            yp_ref[pl.ds(r0, 32), :] = blk


def _l2_fwd(u, yp_ref, g_ref, wp_ref, tw_ref):
    c = u // 8
    kp = u % 8
    base = pl.multiple_of(u * 512, 512)
    ys = [yp_ref[pl.ds(base + al * 128, 128), :] for al in range(4)]
    tws = [None] + [(tw_ref[(al * kp) % 32], tw_ref[32 + (al * kp) % 32]) for al in range(1, 4)]
    outs = [[None] * 8 for _ in range(4)]
    for g in range(8):
        uu = []
        for al in range(4):
            re, im = ys[al][16 * g:16 * g + 8], ys[al][16 * g + 8:16 * g + 16]
            if al > 0:
                cs, sn = tws[al]
                re, im = re * cs + im * sn, im * cs - re * sn
            uu.append((re, im))
        o = _fft4(uu, False)
        for kpp in range(4):
            outs[kpp][g] = jnp.concatenate([o[kpp][0], o[kpp][1]], axis=0)
    vsl = []
    for kpp in range(4):
        k1 = kp + 8 * kpp
        yw = jnp.concatenate(outs[kpp], axis=0).astype(BF)
        gf = _unpack(g_ref[pl.ds(pl.multiple_of((kp * 8 + kpp) * 64, 64), 64), :])
        xx = _dot(gf, yw)
        ww = wp_ref[pl.ds(pl.multiple_of((c * 16 + kp // 2 + 4 * kpp) * 128, 128), 128), :]
        w = pltpu.bitcast((ww << (16 - 16 * (kp % 2))) & -65536, F32)
        vs = []
        for g in range(8):
            xr, xi = xx[16 * g:16 * g + 8], xx[16 * g + 8:16 * g + 16]
            wr, wi = w[16 * g:16 * g + 8], w[16 * g + 8:16 * g + 16]
            vs += [xr * wr - xi * wi, xr * wi + xi * wr]
        vsl.append(jnp.concatenate(vs, axis=0).astype(BF))
    return vsl


def _l2_inv(u, vsl, g_ref):
    kp = u % 8
    us = []
    for kpp in range(4):
        gi = _unpack(g_ref[pl.ds(pl.multiple_of((kp * 8 + 4 + kpp) * 64, 64), 64), :])
        us.append(_dot(gi, vsl[kpp]))
    return us


def _l2_fin(u, us, up_ref):
    base = pl.multiple_of(u * 512, 512)
    res = [[None] * 8 for _ in range(4)]
    for g in range(8):
        o = _fft4([(us[kpp][16 * g:16 * g + 8], us[kpp][16 * g + 8:16 * g + 16]) for kpp in range(4)], True)
        for al in range(4):
            res[al][g] = jnp.concatenate([o[al][0], o[al][1]], axis=0)
    for al in range(4):
        up_ref[pl.ds(base + al * 128, 128), :] = jnp.concatenate(res[al], axis=0)


def _l3_a(i, up_ref, mi_ref, tw_ref, idx_ref):
    al = i // 4
    bc = i % 4
    vs = [None] * 3
    for c in (2, 0, 1):
        u = []
        for kp in range(8):
            r0 = pl.multiple_of(((c * 8 + kp) * 4 + al) * 128 + 32 * bc, 32)
            blk = up_ref[pl.ds(r0, 32), :]
            re = jnp.concatenate([blk[0:8], blk[16:24]], axis=0)
            im = jnp.concatenate([blk[8:16], blk[24:32]], axis=0)
            if kp > 0:
                m = (al * kp) % 32
                cs = tw_ref[m]
                sn = tw_ref[32 + m]
                re, im = re * cs - im * sn, im * cs + re * sn
            u.append((re, im))
        o = _fft8(u, True)
        zr = jnp.concatenate([o[j][0] for j in range(8)], axis=0)
        zi = jnp.concatenate([o[j][1] for j in range(8)], axis=0)
        if c == 2:
            lane = jax.lax.broadcasted_iota(I32, (128, 128), 1)
            used = functools.reduce(lambda a_, b_: a_ | b_, [(lane >= lo_) & (lane < hi_) for lo_, hi_ in _C0RANGES])
            zp = jnp.take_along_axis(zi, jnp.broadcast_to(idx_ref[32:33, :], (128, 128)), axis=1)
            lhs = jnp.where(used, zr, zp).astype(BF)
            vs[c] = _dot(lhs, _unpack(mi_ref[:, 768:896]))
            continue
        sg = pltpu.bitcast(idx_ref[40 + 8 * c:48 + 8 * c, :], F32)
        zi = zi * jnp.concatenate([sg] * 16, axis=0)
        p1 = _dot(zr.astype(BF), _unpack(mi_ref[:, 384 * c:384 * c + 128]))
        p2 = _dot(zi.astype(BF), _unpack(mi_ref[:, 384 * c + 128:384 * c + 256]))
        p3 = _dot((zr + zi).astype(BF), _unpack(mi_ref[:, 384 * c + 256:384 * c + 384]))
        vs[c] = jnp.concatenate([p1 - p2, p3 - p1 - p2], axis=1)
    return vs


def _l3_b(i, vs, out_ref):
    v1r, v1i = vs[0][:, :128], vs[0][:, 128:]
    v2r, v2i = vs[1][:, :128], vs[1][:, 128:]
    v0 = vs[2]
    pa = C1 * v1r + C2 * v2r
    pb = C2 * v1r + C1 * v2r
    qa = S1 * v1i + S2 * v2i
    qb = S2 * v1i - S1 * v2i
    ea = v0 + pa
    eb = v0 + pb
    ys = [v0 + v1r + v2r, ea - qa, eb - qb, eb + qb, ea + qa]
    y = jnp.concatenate(ys, axis=1).astype(BF)
    for j in range(8):
        out_ref[j, i, :, 0:D] = y[16 * j:16 * j + 16]


def _wprep_iter(hi3, w_ref, idx_ref, wp_ref, part):
    lane = jax.lax.broadcasted_iota(I32, (128, 128), 1)
    sub = jax.lax.broadcasted_iota(I32, (8, 128), 0)
    srt = []
    for t in range(3):
        halves = []
        for kt in range(2):
            k0 = pl.multiple_of(hi3 * 256 + kt * 128, 128)
            if t < 2:
                blk = w_ref[128 * t:128 * t + 128, pl.ds(k0, 128)]
            else:
                blk = jnp.concatenate([w_ref[256:DF, pl.ds(k0, 128)], jnp.zeros((384 - DF, 128), BF)], axis=0)
            halves.append(pltpu.bitcast(blk.T, I32))
        words = jnp.concatenate(halves, axis=0)
        idx = jnp.broadcast_to(idx_ref[8 * t:8 * t + 1, :], (128, 128))
        srt.append(jnp.take_along_axis(words, idx, axis=1))
    for c in range(3):
        if c == 0:
            t = jnp.where(lane < 51, srt[0], jnp.where(lane < 102, srt[1], srt[2]))
        elif c == 1:
            t = jnp.where((lane >= 51) & (lane < 102), srt[0], jnp.where((lane >= 25) & (lane < 51), srt[2], srt[1]))
        else:
            t = jnp.where(lane >= 102, srt[0], jnp.where(lane < 51, srt[1], srt[2]))
        for bit4 in range(2):
            v = [t[8 * (bit4 + 2 * m):8 * (bit4 + 2 * m) + 8] for m in range(8)]
            for s_ in range(3):
                sh = 1 << s_
                nv = [None] * 8
                lo_mask = (sub & sh) == 0
                for m in range(8):
                    if m & sh:
                        continue
                    a_, b_ = v[m], v[m + sh]
                    ra = pltpu.roll(a_, 8 - sh, axis=0)
                    rb = pltpu.roll(b_, sh, axis=0)
                    nv[m] = jnp.where(lo_mask, a_, rb)
                    nv[m + sh] = jnp.where(lo_mask, ra, b_)
                v = nv
            for mp in range(8):
                rr = pl.multiple_of((c * 16 + mp + 8 * bit4) * 128 + 16 * hi3 + 8 * part, 8)
                wp_ref[pl.ds(rr, 8), :] = v[mp]


def _kproj(i, xb_ref, wk_ref, k32_ref, half):
    r0 = pl.multiple_of(i * 128, 128)
    c0, c1 = ((0, 384), (384, 640))[half]
    z = _dot(xb_ref[pl.ds(r0, 128), :], _unpack(wk_ref[:, c0:c1]))
    k32_ref[pl.ds(pl.multiple_of(i * 128 + 64, 64), 128), c0:c1] = z.astype(BF)


NWIN = 13


def _kpair(i, k32_ref, kp32_ref):
    lane = jax.lax.broadcasted_iota(I32, (128, 128), 1)
    r0 = pl.multiple_of(i * 128, 128)
    rr = pl.multiple_of(i * 256, 256)
    lo = [pltpu.bitcast(k32_ref[pl.ds(rr, 256), 128 * t:128 * t + 128], I32) for t in range(5)]
    hi = [pltpu.bitcast(k32_ref[pl.ds(rr + 64, 256), 128 * t:128 * t + 128], I32) for t in range(5)]
    for m in range(NWIN):
        t0, off = divmod(48 * m, 128)
        if off + 64 <= 128:
            a, b = lo[t0], hi[t0]
        else:
            a = jnp.where(lane >= off, lo[t0], lo[t0 + 1])
            b = jnp.where(lane >= off, hi[t0], hi[t0 + 1])
        sa, sb = (128 - off) % 128, (64 - off) % 128
        if sa:
            a = pltpu.roll(a, sa, axis=1)
        if sb:
            b = pltpu.roll(b, sb, axis=1)
        kp32_ref[pl.ds(r0, 128), 128 * m:128 * m + 128] = jnp.where(lane < 64, a, b)


def _qproj(i, xb_ref, wqt_ref, qt32_ref, half):
    r0 = pl.multiple_of(i * 128, 128)
    w = _unpack(wqt_ref[160 * half:160 * half + 160, :])
    z = _dot_nt(w, xb_ref[pl.ds(r0, 128), :])
    qt32_ref[320 * half:320 * half + 320, pl.ds(r0, 128)] = (z * QSCALE).astype(BF)


def _vproj(i, xb_ref, wvt_ref, vt32_ref, half):
    r0 = pl.multiple_of(i * 128, 128)
    w = _unpack(wvt_ref[160 * half:160 * half + 160, :])
    z = _dot_nt(w, xb_ref[pl.ds(r0, 128), :])
    ones8 = jnp.where(jax.lax.broadcasted_iota(I32, (8, 128), 0) == 0, 1.0, 0.0).astype(F32)
    pieces = []
    for m in range(8):
        pieces += [z[40 * m:40 * m + 24], ones8, z[40 * m + 16:40 * m + 40], ones8]
    vt32_ref[512 * half:512 * half + 512, pl.ds(r0, 128)] = jnp.concatenate(pieces, axis=0).astype(BF)


def _get_wq(qt32_ref, h, q0):
    m = DH * h // 48
    p0 = (DH * h - 48 * m) // 2
    rowi = jax.lax.broadcasted_iota(I32, (32, 128), 0)
    lane = jax.lax.broadcasted_iota(I32, (32, 128), 1)
    w = pltpu.bitcast(qt32_ref[48 * m:48 * m + 64, pl.ds(q0, 128)], I32)
    rm = (rowi >= p0) & (rowi < p0 + DH // 2)
    lo = jnp.where(rm & (lane < 64), w, 0)
    hi = jnp.where(rm & (lane >= 64), w, 0)
    return m, _unpack(jnp.concatenate([lo, hi], axis=0))


def _rows0(nb):
    return (0, 192, 64, 0)[nb]


def _init_bias(bias_ref):
    r = jax.lax.broadcasted_iota(I32, (64, 128), 0)
    lane = jax.lax.broadcasted_iota(I32, (64, 128), 1)
    upper = r > (lane & 63)
    bias_ref[0:64, :] = jnp.where(upper, 0.0, NEG)
    bias_ref[64:128, :] = jnp.where(upper, NEG, 0.0)
    bias_ref[128:136, :] = jnp.where(lane[0:8] >= 64, 0.0, NEG)


def _s1(j, g, nb, buf, z, kp32_ref, qt32_ref, bias_ref):
    q0 = pl.multiple_of(j * 128, 128)
    r0 = _rows0(nb)
    zz = pl.multiple_of(z * 8, 8)
    cuts = [c for c in (64, 192) if c > r0]
    edges = [r0] + cuts + [320]
    ms = [None] * 4
    for ra, rb in zip(edges[:-1], edges[1:]):
        for a in range(4):
            h = 4 * g + a
            m, wq = _get_wq(qt32_ref, h, q0)
            k0 = pl.multiple_of(j * 64 - 96 + ra // 2, 8)
            kb = _unpack(kp32_ref[pl.ds(k0, (rb - ra) // 2), 128 * m:128 * m + 128])
            s = _dot(kb, wq)
            parts = []
            for v in range(ra // 8, rb // 8):
                sb = s[8 * v - ra:8 * v - ra + 8]
                b, vv = divmod(v, 8)
                if b == 0:
                    sb = sb + bias_ref[8 * vv:8 * vv + 8, :]
                elif b == 4:
                    sb = sb + bias_ref[64 + 8 * vv:64 + 8 * vv + 8, :]
                elif nb < 3 and 64 * b == r0:
                    sb = sb + bias_ref[128:136, :]
                parts.append(sb)
            s = jnp.concatenate(parts, axis=0)
            buf[pl.ds(zz + a * 320 + ra, rb - ra), :] = s
            mb = jnp.max(s.reshape((rb - ra) // 8, 8, 128), axis=0)
            ms[a] = mb if ms[a] is None else jnp.maximum(ms[a], mb)
    return [jnp.max(m_, axis=0, keepdims=True) for m_ in ms]


def _s2(j, g, nb, buf, z, ms, vt32_ref, aot_ref):
    sub = jax.lax.broadcasted_iota(I32, (8, 128), 0)
    lane = jax.lax.broadcasted_iota(I32, (8, 128), 1)
    lo = lane < 64
    r0 = _rows0(nb)
    zz = pl.multiple_of(z * 8, 8)
    cache = {}

    def sh(a, v):
        if (a, v) not in cache:
            cache[(a, v)] = jnp.exp2(buf[pl.ds(zz + a * 320 + 8 * v, 8), :] - ms[a])
        return cache[(a, v)]

    def pun(a, b):
        un = []
        for v in range(16 * b, 16 * b + 16):
            if v < 8:
                un.append(jnp.where(lo, sh(a, v), 0.0))
            elif v < 40:
                un.append(jnp.where(lo, sh(a, v), sh(a, v - 8)))
            else:
                un.append(jnp.where(lo, 0.0, sh(a, v - 8)))
        return jnp.concatenate(un, axis=0).astype(BF)

    acc = [None] * 4
    order = [(a, b) for b in range(3 - nb, 3) for a in range(4)]
    for a, b in order:
        h = 4 * g + a
        k0 = pl.multiple_of((j - 2 + b) * 128, 128)
        vt = vt32_ref[32 * h:32 * h + 32, pl.ds(k0, 128)]
        d = _dot(vt, pun(a, b))
        acc[a] = d if acc[a] is None else acc[a] + d
    os_ = [o[0:24, :] * (1.0 / o[24:25, :]) for o in acc]
    blks = []
    for a in (0, 2):
        e, od = os_[a], os_[a + 1]
        blks += [e[0:16], jnp.where(sub < 4, e[16:24], od[0:8]), od[8:24]]
    aot_ref[80 * g:80 * g + 80, :] = jnp.concatenate(blks, axis=0)


def _outproj(j, aot_ref, wo_ref, out_ref):
    ao = jnp.concatenate([aot_ref[128 * t:128 * t + 128, :].T for t in range(5)], axis=1).astype(BF)
    z = _dot(ao, wo_ref[...])
    out_ref[j // 2, pl.ds(pl.multiple_of((j % 2) * 8, 8), 8), :, D:2 * D] = z.astype(BF).reshape(8, 16, D)


def _kernel(idx_hbm, xa_hbm, wr_hbm, wi_hbm, xb_hbm, wqkv_hbm, wo_hbm, g_hbm, mf_hbm, mi_hbm, out_hbm,
            xa_v, wr_v, wi_v, xb_v, wq_v, wk_v, wv_v, wo_v, g_v, mf_ref, mi_ref,
            wqt_v, wvt_v, wk32, k32, kp32, qt32, vt32, aot, aot2, sbuf0, sbuf1, sbuf2, sbuf3, bias,
            yp, up, wp, ostage, idx_ref, tw_ref, z_ref, sems, csem, gsem, osem):
    def cp(src, dst, k):
        return pltpu.make_async_copy(src, dst, sems.at[k])

    c_wk = cp(wqkv_hbm.at[:, D:2 * D], wk_v, 0)
    c_wq = cp(wqkv_hbm.at[:, 0:D], wq_v, 1)
    c_wv = cp(wqkv_hbm.at[:, 2 * D:3 * D], wv_v, 2)
    c_wo = cp(wo_hbm, wo_v, 3)
    c_mf = cp(mf_hbm, mf_ref, 4)
    c_mi = cp(mi_hbm, mi_ref, 5)
    c_idx = cp(idx_hbm, idx_ref, 6)

    def chunk(i):
        r = pl.ds(pl.multiple_of(i * 256, 256), 256)
        m = pl.ds(pl.multiple_of(i * 2, 2), 2)
        return (pltpu.make_async_copy(xb_hbm.at[r], xb_v.at[r], csem.at[4 * i]),
                pltpu.make_async_copy(xa_hbm.at[:, m], xa_v.at[:, m], csem.at[4 * i + 1]),
                pltpu.make_async_copy(wr_hbm.at[:, r], wr_v.at[:, r], csem.at[4 * i + 2]),
                pltpu.make_async_copy(wi_hbm.at[:, r], wi_v.at[:, r], csem.at[4 * i + 3]))

    def gchunk(kp):
        r = pl.ds(pl.multiple_of(kp * 512, 512), 512)
        return pltpu.make_async_copy(g_hbm.at[r], g_v.at[r], gsem.at[kp])

    def loop(n, pre, f, post, u=1):
        def group(i0):
            for t in range(u):
                pre(i0 + t)
            for t in range(u):
                f(i0 + t)
            for t in range(u):
                post(i0 + t)
        if u >= n:
            group(0)
        else:
            jax.lax.fori_loop(0, n // u, lambda i, c_: (group(i * u), c_)[1], 0)

    def none(i):
        pass

    c_wk.start()
    ch0 = chunk(0)
    ch0[0].start()
    c_mf.start()
    c_idx.start()
    for c_ in ch0[1:]:
        c_.start()

    for n in range(64):
        tw_ref[n] = float(_TW[n])
    for n in range(NZ):
        z_ref[n] = 0
    k32[0:64, :] = jnp.zeros((64, D), BF)
    _init_bias(bias)

    c_wk.wait()
    for c_ in chunk(1):
        c_.start()
    wk32[...] = pltpu.bitcast(wk_v[...], I32)
    c_mf.wait()
    c_idx.wait()

    def pre1(i):
        @pl.when(i < 6)
        def _():
            for c_ in chunk(i + 2):
                c_.start()

        pl.when(i == 3)(c_wq.start)
        pl.when(i == 6)(c_wq.wait)
        pl.when(i == 6)(gchunk(0).start)
        pl.when(i == 7)(gchunk(1).start)
        for c_ in chunk(i):
            c_.wait()

    def ph1(i):
        _wprep_iter(i, wr_v, idx_ref, wp, 0)
        _wprep_iter(i, wi_v, idx_ref, wp, 1)
        for t in range(2):
            _kproj(2 * i + t, xb_v, wk32, k32, 0)
            zs = _l1_a(2 * i + t, xa_v, mf_ref, idx_ref)
            _l1_b(2 * i + t, zs, tw_ref, yp)
            _kproj(2 * i + t, xb_v, wk32, k32, 1)
    loop(7, pre1, ph1, none)
    pre1(7)
    ph1(7)

    wqt_v[...] = pltpu.bitcast(wq_v[...].T, I32)

    def pre2(kp):
        @pl.when(kp < 6)
        def _():
            gchunk(kp + 2).start()

        pl.when(kp == 2)(c_wv.start)
        pl.when(kp == 4)(c_mi.start)
        pl.when(kp == 5)(c_wo.start)
        pl.when(kp == 5)(c_wv.wait)
        pl.when(kp == 6)(c_mi.wait)
        gchunk(kp).wait()

    def ph2pair(k0):
        k1 = k0 + 1
        qp = lambda t, h: _qproj(t, xb_v, wqt_v, qt32, h)
        _kpair(k0, k32, kp32)
        _kpair(k1, k32, kp32)
        qp(2 * k0, 0)
        sa = [_l2_fwd(c * 8 + k0, yp, g_v, wp, tw_ref) for c in range(3)]
        qp(2 * k0, 1)
        sb = [_l2_fwd(c * 8 + k1, yp, g_v, wp, tw_ref) for c in range(3)]
        qp(2 * k0 + 1, 0)
        ua = [_l2_inv(c * 8 + k0, sa[c], g_v) for c in range(3)]
        for c in range(3):
            _l2_fin(c * 8 + k0, ua[c], up)
        qp(2 * k0 + 1, 1)
        qp(2 * k1, 0)
        ub = [_l2_inv(c * 8 + k1, sb[c], g_v) for c in range(3)]
        for c in range(3):
            _l2_fin(c * 8 + k1, ub[c], up)
        qp(2 * k1, 1)
        qp(2 * k1 + 1, 0)
        qp(2 * k1 + 1, 1)

    def it2(ii, c_):
        pre2(2 * ii)
        pre2(2 * ii + 1)
        ph2pair(2 * ii)
        return c_
    jax.lax.fori_loop(0, 3, it2, 0)
    pre2(6)
    pre2(7)
    ph2pair(6)

    wvt_v[...] = pltpu.bitcast(wv_v[...].T, I32)

    def out_a(i):
        m = pl.ds(pl.multiple_of(i * 2, 2), 2)
        return pltpu.make_async_copy(ostage.at[:, m, :, 0:D], out_hbm.at[:, m, :, 0:D], osem.at[0])

    def ph3(i):
        for t in range(2):
            _vproj(2 * i + t, xb_v, wvt_v, vt32, 0)
            va = _l3_a(2 * i + t, up, mi_ref, tw_ref, idx_ref)
            _vproj(2 * i + t, xb_v, wvt_v, vt32, 1)
            _l3_b(2 * i + t, va, ostage)

    loop(8, none, ph3, lambda i: out_a(i).start(), 4)

    c_wo.wait()
    bufs = (sbuf0, sbuf1)
    bufs2 = (sbuf2, sbuf3)
    zc = [0]

    def oz():
        zc[0] += 1
        return z_ref[zc[0] % NZ]

    def out_copy(j):
        m = pl.ds(pl.multiple_of((j % 2) * 8, 8), 8)
        return pltpu.make_async_copy(ostage.at[j // 2, m, :, D:2 * D], out_hbm.at[j // 2, m, :, D:2 * D], osem.at[1])

    def body(j, nb, nb_next, ms, ao, ops, last):
        for g in range(8):
            if g < 7:
                ms_n = _s1(j, g + 1, nb, bufs[(g + 1) % 2], oz(), kp32, qt32, bias)
            elif not last:
                ms_n = _s1(j + 1, 0, nb_next, bufs[0], oz(), kp32, qt32, bias)
            else:
                ms_n = None
            if g == 0:
                for jo, aob in ops:
                    _outproj(jo, aob, wo_v, ostage)
                    out_copy(jo).start()
            _s2(j, g, nb, bufs[g % 2], oz(), ms, vt32, ao)
            ms = ms_n
        return ms

    ms = _s1(0, 0, 1, bufs[0], oz(), kp32, qt32, bias)
    msa = ms
    msb = _s1(1, 0, 2, bufs2[0], oz(), kp32, qt32, bias)
    for g in range(8):
        if g < 7:
            nb_ = _s1(1, g + 1, 2, bufs2[(g + 1) % 2], oz(), kp32, qt32, bias)
        _s2(0, g, 1, bufs[g % 2], oz(), msa, vt32, aot)
        if g < 7:
            na = _s1(0, g + 1, 1, bufs[(g + 1) % 2], oz(), kp32, qt32, bias)
        else:
            ms = _s1(2, 0, 3, bufs[0], oz(), kp32, qt32, bias)
        _s2(1, g, 2, bufs2[g % 2], oz(), msb, vt32, aot2)
        msa, msb = na, nb_

    def two(jj, m):
        m = body(2 * jj, 3, 3, list(m), aot, [(2 * jj - 2, aot), (2 * jj - 1, aot2)], False)
        return tuple(body(2 * jj + 1, 3, 3, m, aot2, [], False))
    ms = jax.lax.fori_loop(1, 7, two, tuple(ms))
    ms = body(14, 3, 3, list(ms), aot, [(12, aot), (13, aot2)], False)
    body(15, 3, 3, list(ms), aot2, [(14, aot)], True)
    _outproj(15, aot2, wo_v, ostage)
    out_copy(15).start()
    for j in range(8):
        out_a(j).wait()
    for j in range(16):
        out_copy(j).wait()


@jax.jit
def pallas_concat_heads__spectral_gfnet__sliding_block__prompt_kernel(
    A_x: jax.Array,
    A_w_r: jax.Array,
    A_w_i: jax.Array,
    B_x: jax.Array,
    B_wqkv: jax.Array,
    B_wo: jax.Array,
):
    hbm = pl.BlockSpec(memory_space=pltpu.HBM)
    out = pl.pallas_call(
        _kernel,
        out_shape=jax.ShapeDtypeStruct((8, 16, 16, 2 * D), BF),
        in_specs=[hbm] * 10,
        out_specs=hbm,
        scratch_shapes=[
            pltpu.VMEM((8, 16, 16, D), BF), pltpu.VMEM((DF, S), BF), pltpu.VMEM((DF, S), BF), pltpu.VMEM((S, D), BF),
            pltpu.VMEM((D, D), BF), pltpu.VMEM((D, D), BF), pltpu.VMEM((D, D), BF), pltpu.VMEM((D, D), BF),
            pltpu.VMEM((32 * 128, 128), I32), pltpu.VMEM((192, 384), I32), pltpu.VMEM((64, 896), I32),
            pltpu.VMEM((D // 2, D), I32), pltpu.VMEM((D // 2, D), I32), pltpu.VMEM((D // 2, D), I32),
            pltpu.VMEM((S + 64, D), BF), pltpu.VMEM((S // 2, NWIN * 128), I32), pltpu.VMEM((D, S), BF), pltpu.VMEM((1024, S), BF),
            pltpu.VMEM((D, 128), F32), pltpu.VMEM((D, 128), F32),
            pltpu.VMEM((4 * 320, 128), F32), pltpu.VMEM((4 * 320, 128), F32),
            pltpu.VMEM((4 * 320, 128), F32), pltpu.VMEM((4 * 320, 128), F32), pltpu.VMEM((136, 128), F32),
            pltpu.VMEM((96 * 128, 128), F32), pltpu.VMEM((96 * 128, 128), F32), pltpu.VMEM((48 * 128, 128), I32),
            pltpu.VMEM((8, 16, 16, 2 * D), BF),
            pltpu.VMEM((56, 128), I32), pltpu.SMEM((64,), F32), pltpu.SMEM((NZ,), I32),
            pltpu.SemaphoreType.DMA((7,)), pltpu.SemaphoreType.DMA((32,)), pltpu.SemaphoreType.DMA((8,)),
            pltpu.SemaphoreType.DMA((2,)),
        ],
        compiler_params=pltpu.CompilerParams(vmem_limit_bytes=110 * 1024 * 1024),
    )(_IDX,
      A_x.reshape(8, 16, 16, D), A_w_r.T, A_w_i.T, B_x.reshape(S, D), B_wqkv, B_wo, _G, _MF, _MI)
    return out.reshape(1, S, 2 * D)
```
